```python
import jax
import jax.numpy as jnp

def _softmax(x, axis=-1):
    return jax.nn.softmax(x, axis=axis)
def _gelu(x):
    return jax.nn.gelu(x, approximate=True)
def _silu(x):
    return jax.nn.silu(x)
def _sigmoid(x):
    return jax.nn.sigmoid(x)
def _layernorm(x, axis=-1, eps=1e-5):
    m = jnp.mean(x, axis=axis, keepdims=True)
    v = jnp.var(x, axis=axis, keepdims=True)
    return (x - m) / jnp.sqrt(v + eps)
def _scatter_add(tgt, idx, src, axis=0):
    return tgt.at[idx].add(src)
def _segment_sum(src, seg, n):
    return jax.ops.segment_sum(src, seg, n)
class _Rng:
    def __init__(self, key):
        self._k = key
    def _next(self):
        self._k, sub = jax.random.split(self._k)
        return sub
    def normal(self, shape):
        return jax.random.normal(self._next(), shape, dtype=jnp.bfloat16)
    def randint(self, lo, hi, shape):
        return jax.random.randint(self._next(), shape, lo, hi, dtype=jnp.int32)
    def uniform(self, shape, lo=0.0, hi=1.0):
        return jax.random.uniform(self._next(), shape, jnp.bfloat16, lo, hi)
    def permutation(self, n):
        return jax.random.permutation(self._next(), n)


kernel_name = 'standalone__depthwise_separable__vision'

def setup_inputs():
    _rng = _Rng(jax.random.key(int.from_bytes(__import__("os").urandom(4), "little")))
    _w = (lambda a: (lambda t: t.astype(jnp.bfloat16) if jnp.issubdtype(t.dtype, jnp.floating) else t)(jnp.asarray(a)))
    H = W = 384
    C = 384
    k = 1
    return {
        "x": _w((lambda *s: _rng.normal(s) * 0.05)(1, H, W, C)),
        "dw": _w((lambda *s: _rng.normal(s) * 0.05)(k, k, C)),
        "pw": _w((lambda *s: _rng.normal(s) * 0.05)(C, C)),
    }

def reference(x, dw, pw):
    B, H, W, C = x.shape
    k = dw.shape[0]
    pad = k // 2
    xp = jnp.pad(x, ((0,0),(pad,pad),(pad,pad),(0,0)))
    out = jnp.zeros_like(x)
    for i in range(k):
        for j in range(k):
            out = out + xp[:, i:i+H, j:j+W, :] * dw[i, j][None, None, None, :]
    return jnp.einsum('bhwc,cd->bhwd', out, pw)
```

```python
import jax
import jax.numpy as jnp
from jax import lax
import jax.experimental.pallas as pl
import jax.experimental.pallas.tpu as pltpu

_K = 8
_L = 2048
_TS = 128
_S = 16
_TPC = 4
_I0 = 80
_NB = 3
_BT = 2
_TAIL = 64


@jax.jit
def pallas_standalone__depthwise_separable__vision_kernel(
    x: jax.Array,
    dw: jax.Array,
    pw: jax.Array,
):
    B, H, W, C = x.shape
    assert dw.shape == (1, 1, C) and pw.shape == (C, C)
    M = B * H * W
    k, L, ts, s, tpc, i0, NB, bt, tail = _K, _L, _TS, _S, _TPC, _I0, _NB, _BT, _TAIL
    G = M // (k * L)
    assert G * k * L == M
    tpg = L // ts
    n = G * tpg
    nr = n // tpc
    cpg = tpg // tpc
    rc = tpc * ts
    rb = bt * ts
    bpg = L // rb
    nb = n // bt
    n2 = n - i0
    assert tpg % tpc == 0 and tpg % bt == 0 and i0 % tpc == 0 and NB + n2 <= nb
    assert all((NB + j + 1) * bt <= i0 + j for j in range(n2))

    def aligned(v, m):
        return v if isinstance(v, int) else pl.multiple_of(v, m)

    def kernel(x_hbm, dw_hbm, pw_hbm, o_hbm, buf, dw_ref, pw_ref, rsems, wsems, psems):
        def read(c, lo=0, size=rc, sem=None):
            g = c // cpg
            rows = pl.ds(aligned((c % cpg) * rc, rc) + lo, size)
            return pltpu.make_async_copy(
                x_hbm.at[g, :, rows, :], buf.at[g, :, rows, :],
                rsems.at[c] if sem is None else sem)

        def write(b, lo, size):
            g = b // bpg
            rows = pl.ds(aligned((b % bpg) * rb + lo, s), size)
            return pltpu.make_async_copy(
                buf.at[g, :, rows, :], o_hbm.at[g, :, rows, :], wsems.at[b % NB])

        def write_start(b):
            for d in range(rb // s):
                write(b, d * s, s).start()

        def write_wait(b):
            write(b, 0, rb).wait()

        def compute(t):
            g = t // tpg
            rows = pl.ds(pl.multiple_of((t % tpg) * ts, ts), ts)
            xt = buf[g, :, rows, :].reshape(k * ts, C)
            y = jnp.dot(xt * dw_ref[0], pw_ref[...],
                        preferred_element_type=jnp.float32)
            buf[g, :, rows, :] = y.astype(buf.dtype).reshape(k, ts, C)

        copy_dw = pltpu.make_async_copy(dw_hbm, dw_ref, psems.at[0])
        copy_pw = pltpu.make_async_copy(pw_hbm, pw_ref, psems.at[1])
        read(0).start()
        copy_dw.start()
        copy_pw.start()

        def issue_read(c, carry):
            read(c).start()
            return carry

        lax.fori_loop(1, nr - 1, issue_read, 0)
        last_a = read(nr - 1, 0, rc - tail)
        last_b = read(nr - 1, rc - tail, tail, psems.at[2])
        last_a.start()

        def issue_tail(i, carry):
            last_b.start()
            return carry

        lax.fori_loop(0, 1, issue_tail, 0)
        copy_dw.wait()
        copy_pw.wait()

        def phase1(t, carry):
            @pl.when(t % tpc == 0)
            def _():
                read(t // tpc).wait()

            compute(t)
            return carry

        lax.fori_loop(0, i0, phase1, 0)
        for c in range(i0 // tpc, nr - 1):
            read(c).wait()
        last_a.wait()
        for b in range(NB):
            write_start(b)
        last_b.wait()

        def phase2(j, carry):
            write_wait(j)
            write_start(j + NB)
            compute(i0 + j)
            return carry

        lax.fori_loop(0, n2, phase2, 0)

        def drain(j, carry):
            write_wait(j)
            write_start(j + NB)
            return carry

        lax.fori_loop(n2, nb - NB, drain, 0)
        for b in range(nb - NB, nb):
            write_wait(b)

    out = pl.pallas_call(
        kernel,
        in_specs=[pl.BlockSpec(memory_space=pl.ANY)] * 3,
        out_specs=pl.BlockSpec(memory_space=pl.ANY),
        out_shape=jax.ShapeDtypeStruct((G, k, L, C), x.dtype),
        scratch_shapes=[
            pltpu.VMEM((G, k, L, C), x.dtype),
            pltpu.VMEM(dw.shape, dw.dtype),
            pltpu.VMEM(pw.shape, pw.dtype),
            pltpu.SemaphoreType.DMA((nr,)),
            pltpu.SemaphoreType.DMA((NB,)),
            pltpu.SemaphoreType.DMA((3,)),
        ],
        compiler_params=pltpu.CompilerParams(vmem_limit_bytes=124 * 1024 * 1024),
    )(x.reshape(G, k, L, C), dw, pw)
    return out.reshape(B, H, W, C)
```

```python
import jax
import jax.numpy as jnp
from jax import lax
import jax.experimental.pallas as pl
import jax.experimental.pallas.tpu as pltpu

_K = 6
_L = 2048
_TS = 128
_I0 = 100
_FS = 8
_NPIN = 14
_BS = 32
_AHEAD = 3
_RS = 64
_WS = 16
_NB = 2


def _pin_positions(n, rows):
    pos = [round(i * (2 * rows - 16) / (n - 2) / 16) * 16 for i in range(n - 1)]
    return [(0, p) if p < rows else (2, p - rows) for p in pos]


@jax.jit
def pallas_standalone__depthwise_separable__vision_kernel(
    x: jax.Array,
    dw: jax.Array,
    pw: jax.Array,
):
    B, H, W, C = x.shape
    assert dw.shape == (1, 1, C) and pw.shape == (C, C) and C == 384
    k, L, ts, i0, fs, npin = _K, _L, _TS, _I0, _FS, _NPIN
    bs, ahead, rs, ws, NB = _BS, _AHEAD, _RS, _WS, _NB
    G = B * H * W // (k * L)
    assert G * k * L == B * H * W
    Q = L // ts
    n = G * Q
    n2 = n - i0
    per_tile = ts // fs
    full, left = divmod(i0 * npin, per_tile)
    nb_a, nb = i0 // 2, n // 2
    ring = ahead + 1
    assert i0 % 2 == 0 and full + 1 < n2 and nb_a + NB <= NB + n2 <= nb
    assert all((NB + j + 1) * 2 <= i0 + j for j in range(n2))
    pins = _pin_positions(npin, k * ts)

    def aligned(v):
        return v if isinstance(v, int) else pl.multiple_of(v, 8)

    def div(a, b):
        return a // b if isinstance(a, int) else lax.div(a, b)

    def rem(a, b):
        return a % b if isinstance(a, int) else lax.rem(a, b)

    def kernel(x_hbm, dw_hbm, pw_hbm, o_hbm, buf_a, buf_b, dw_ref, pw_ref, wsems):
        def hbm(ref, t, lo, size):
            return ref.at[div(t, Q), :, pl.ds(aligned(rem(t, Q) * ts + lo), size), :]

        def vmem(buf, slot, lo, size):
            return buf.at[pl.ds(slot * k, k), pl.ds(aligned(lo), size), :]

        def write(in_a, b, half, lo, size):
            t = 2 * b + half
            src = vmem(buf_a, t, lo, size) if in_a else vmem(buf_b, t - i0, lo, size)
            return pltpu.make_async_copy(
                src, hbm(o_hbm, t, lo, size), wsems.at[rem(b, NB)])

        def write_start(in_a, b):
            for half in range(2):
                for lo in range(0, ts, ws):
                    write(in_a, b, half, lo, ws).start()

        def write_wait(in_a, b):
            for half in range(2):
                write(in_a, b, half, 0, ts).wait()

        def compute(buf, slot):
            xt = buf[pl.ds(slot * k, k)].reshape(k * ts, C)
            y = jnp.dot(xt * dw_ref[0], pw_ref[...],
                        preferred_element_type=jnp.float32)
            buf[pl.ds(slot * k, k)] = y.astype(buf.dtype).reshape(k, ts, C)
            return y

        def read_phase(rsems):
            hi_sem, lo_sem, last_sem = (rsems.at[ring + i] for i in range(3))

            def read_a(t, lo, size):
                return pltpu.make_async_copy(
                    hbm(x_hbm, t, lo, size), vmem(buf_a, t, lo, size),
                    rsems.at[rem(t, ring)])

            def read_b(slot, lo, size, sem):
                return pltpu.make_async_copy(
                    hbm(x_hbm, i0 + slot, lo, size), vmem(buf_b, slot, lo, size), sem)

            def start_tile_a(t):
                for lo in range(0, ts, bs):
                    read_a(t, lo, bs).start(priority=1)

            copy_dw = pltpu.make_async_copy(dw_hbm, dw_ref, lo_sem)
            copy_pw = pltpu.make_async_copy(pw_hbm, pw_ref, lo_sem)
            start_tile_a(0)
            copy_dw.start(priority=1)
            copy_pw.start(priority=1)
            for t in range(1, ahead):
                start_tile_a(t)
            copy_dw.wait()
            copy_pw.wait()

            rest = [read_b(full, left * fs, ts - left * fs, lo_sem)]
            rest += [read_b(slot, lo, rs, lo_sem)
                     for slot in range(full + 1, n2 - 1) for lo in range(0, ts, rs)]
            last = read_b(n2 - 1, 0, ts, last_sem)

            def step(t, carry):
                read_a(t, 0, ts).wait()

                @pl.when(t + ahead < i0)
                def _():
                    start_tile_a(t + ahead)

                @pl.when(t + ahead == i0)
                def _():
                    for c in rest + [last]:
                        c.start(priority=1)

                y = compute(buf_a, t)
                for i in range(npin):
                    if i > 0:
                        cb, r = pins[i - 1]
                        buf_b[n2 * k, pl.ds(0, 16), pl.ds(0, 128)] = (
                            y[r:r + 16, cb * 128:(cb + 1) * 128].astype(buf_b.dtype))
                    d = t * npin + i
                    read_b(div(d, per_tile), rem(d, per_tile) * fs, fs,
                           hi_sem).start(priority=0)
                return carry

            lax.fori_loop(0, i0, step, 0)
            whole = buf_b.at[pl.ds(0, full * k)]
            pltpu.make_async_copy(whole, whole, hi_sem).wait()
            if left:
                read_b(full, 0, left * fs, hi_sem).wait()
            for c in rest:
                c.wait()
            for b in range(NB):
                write_start(True, b)
            last.wait()

        pl.run_scoped(read_phase, pltpu.SemaphoreType.DMA((ring + 3,)))

        def step_a(j, carry):
            write_wait(True, j)
            write_start(True, j + NB)
            compute(buf_b, j)
            return carry

        def step_b(j, carry):
            @pl.when(j < nb_a)
            def _():
                write_wait(True, j)

            @pl.when(j >= nb_a)
            def _():
                write_wait(False, j)

            write_start(False, j + NB)
            compute(buf_b, j)
            return carry

        def drain(j, carry):
            write_wait(False, j)
            write_start(False, j + NB)
            return carry

        lax.fori_loop(0, nb_a - NB, step_a, 0)
        lax.fori_loop(nb_a - NB, n2, step_b, 0)
        lax.fori_loop(n2, nb - NB, drain, 0)
        for b in range(nb - NB, nb):
            write_wait(False, b)

    out = pl.pallas_call(
        kernel,
        in_specs=[pl.BlockSpec(memory_space=pl.ANY)] * 3,
        out_specs=pl.BlockSpec(memory_space=pl.ANY),
        out_shape=jax.ShapeDtypeStruct((G, k, L, C), x.dtype),
        scratch_shapes=[
            pltpu.VMEM((i0 * k, ts, C), x.dtype),
            pltpu.VMEM((n2 * k + 1, ts, C), x.dtype),
            pltpu.VMEM(dw.shape, dw.dtype),
            pltpu.VMEM(pw.shape, pw.dtype),
            pltpu.SemaphoreType.DMA((NB,)),
        ],
        compiler_params=pltpu.CompilerParams(vmem_limit_bytes=120 * 1024 * 1024),
    )(x.reshape(G, k, L, C), dw, pw)
    return out.reshape(B, H, W, C)
```

```python
import jax
import jax.numpy as jnp
from jax import lax
import jax.experimental.pallas as pl
import jax.experimental.pallas.tpu as pltpu

_K = 6
_L = 2048
_TS = 128
_I0 = 98
_FS = 8
_NPIN = 15
_BS = 32
_AHEAD = 3
_RS = 64
_WS = 16
_NB = 3
_LEAD = 2


def _pin_positions(n, rows):
    pos = [round(i * (2 * rows - 16) / (n - 2) / 16) * 16 for i in range(n - 1)]
    return [(0, p) if p < rows else (2, p - rows) for p in pos]


@jax.jit
def pallas_standalone__depthwise_separable__vision_kernel(
    x: jax.Array,
    dw: jax.Array,
    pw: jax.Array,
):
    B, H, W, C = x.shape
    assert dw.shape == (1, 1, C) and pw.shape == (C, C) and C == 384
    k, L, ts, i0, fs, npin = _K, _L, _TS, _I0, _FS, _NPIN
    bs, ahead, rs, ws, NB, lead = _BS, _AHEAD, _RS, _WS, _NB, _LEAD
    G = B * H * W // (k * L)
    assert G * k * L == B * H * W
    Q = L // ts
    n = G * Q
    n2 = n - i0
    per_tile = ts // fs
    full, left = divmod(i0 * npin, per_tile)
    nb_a, nb = i0 // 2, n // 2
    ring = ahead + 1
    assert i0 % 2 == 0 and full + 1 < n2 and nb_a <= n2 - lead <= nb - NB
    assert all((NB + j + 1) * 2 <= i0 + lead + j for j in range(n2 - lead))
    pins = _pin_positions(npin, k * ts)

    def aligned(v):
        return v if isinstance(v, int) else pl.multiple_of(v, 8)

    def div(a, b):
        return a // b if isinstance(a, int) else lax.div(a, b)

    def rem(a, b):
        return a % b if isinstance(a, int) else lax.rem(a, b)

    def kernel(x_hbm, dw_hbm, pw_hbm, o_hbm, buf_a, buf_b, dw_ref, pw_ref, wsems):
        def hbm(ref, t, lo, size):
            return ref.at[div(t, Q), :, pl.ds(aligned(rem(t, Q) * ts + lo), size), :]

        def vmem(buf, slot, lo, size):
            return buf.at[pl.ds(slot * k, k), pl.ds(aligned(lo), size), :]

        def write(in_a, b, half, lo, size):
            t = 2 * b + half
            src = vmem(buf_a, t, lo, size) if in_a else vmem(buf_b, t - i0, lo, size)
            return pltpu.make_async_copy(
                src, hbm(o_hbm, t, lo, size), wsems.at[rem(b, NB)])

        def write_start(in_a, b):
            for half in range(2):
                for lo in range(0, ts, ws):
                    write(in_a, b, half, lo, ws).start()

        def write_wait(in_a, b):
            for half in range(2):
                write(in_a, b, half, 0, ts).wait()

        def compute(buf, slot):
            xt = buf[pl.ds(slot * k, k)].reshape(k * ts, C)
            y = jnp.dot(xt * dw_ref[0], pw_ref[...],
                        preferred_element_type=jnp.float32)
            buf[pl.ds(slot * k, k)] = y.astype(buf.dtype).reshape(k, ts, C)
            return y

        def read_phase(rsems):
            hi_sem, lo_sem, last_sem = (rsems.at[ring + i] for i in range(3))

            def read_a(t, lo, size):
                return pltpu.make_async_copy(
                    hbm(x_hbm, t, lo, size), vmem(buf_a, t, lo, size),
                    rsems.at[rem(t, ring)])

            def read_b(slot, lo, size, sem):
                return pltpu.make_async_copy(
                    hbm(x_hbm, i0 + slot, lo, size), vmem(buf_b, slot, lo, size), sem)

            def start_tile_a(t):
                for lo in range(0, ts, bs):
                    read_a(t, lo, bs).start(priority=1)

            copy_dw = pltpu.make_async_copy(dw_hbm, dw_ref, lo_sem)
            copy_pw = pltpu.make_async_copy(pw_hbm, pw_ref, lo_sem)
            start_tile_a(0)
            copy_dw.start(priority=1)
            copy_pw.start(priority=1)
            for t in range(1, ahead):
                start_tile_a(t)
            copy_dw.wait()
            copy_pw.wait()

            rest = [read_b(full, left * fs, ts - left * fs, lo_sem)]
            rest += [read_b(slot, lo, rs, lo_sem)
                     for slot in range(full + 1, n2 - 1) for lo in range(0, ts, rs)]
            last = read_b(n2 - 1, 0, ts, last_sem)

            def step(t, carry):
                read_a(t, 0, ts).wait()

                @pl.when(t + ahead < i0)
                def _():
                    start_tile_a(t + ahead)

                @pl.when(t + ahead == i0)
                def _():
                    for c in rest + [last]:
                        c.start(priority=1)

                y = compute(buf_a, t)
                for i in range(npin):
                    if i > 0:
                        cb, r = pins[i - 1]
                        buf_b[n2 * k, pl.ds(0, 16), pl.ds(0, 128)] = (
                            y[r:r + 16, cb * 128:(cb + 1) * 128].astype(buf_b.dtype))
                    d = t * npin + i
                    read_b(div(d, per_tile), rem(d, per_tile) * fs, fs,
                           hi_sem).start(priority=0)
                return carry

            lax.fori_loop(0, i0, step, 0)
            whole = buf_b.at[pl.ds(0, full * k)]
            pltpu.make_async_copy(whole, whole, hi_sem).wait()
            if left:
                read_b(full, 0, left * fs, hi_sem).wait()
            for c in rest:
                c.wait()
            for b in range(NB):
                write_start(True, b)
            last.wait()

        pl.run_scoped(read_phase, pltpu.SemaphoreType.DMA((ring + 3,)))

        def step_a(j, carry):
            @pl.when(j >= 0)
            def _():
                write_wait(True, j)
                write_start(True, j + NB)

            compute(buf_b, j + lead)
            return carry

        def step_b(j, carry):
            @pl.when(j < nb_a)
            def _():
                write_wait(True, j)

            @pl.when(j >= nb_a)
            def _():
                write_wait(False, j)

            write_start(False, j + NB)
            compute(buf_b, j + lead)
            return carry

        def drain(j, carry):
            write_wait(False, j)
            write_start(False, j + NB)
            return carry

        lax.fori_loop(-lead, nb_a - NB, step_a, 0)
        lax.fori_loop(nb_a - NB, n2 - lead, step_b, 0)
        lax.fori_loop(n2 - lead, nb - NB, drain, 0)
        for b in range(nb - NB, nb):
            write_wait(False, b)

    out = pl.pallas_call(
        kernel,
        in_specs=[pl.BlockSpec(memory_space=pl.ANY)] * 3,
        out_specs=pl.BlockSpec(memory_space=pl.ANY),
        out_shape=jax.ShapeDtypeStruct((G, k, L, C), x.dtype),
        scratch_shapes=[
            pltpu.VMEM((i0 * k, ts, C), x.dtype),
            pltpu.VMEM((n2 * k + 1, ts, C), x.dtype),
            pltpu.VMEM(dw.shape, dw.dtype),
            pltpu.VMEM(pw.shape, pw.dtype),
            pltpu.SemaphoreType.DMA((NB,)),
        ],
        compiler_params=pltpu.CompilerParams(vmem_limit_bytes=120 * 1024 * 1024),
    )(x.reshape(G, k, L, C), dw, pw)
    return out.reshape(B, H, W, C)
```

```python
import jax
import jax.numpy as jnp
from jax import lax
import jax.experimental.pallas as pl
import jax.experimental.pallas.tpu as pltpu

_K = 6
_L = 2048
_TS = 128
_I0 = 98
_FS = 16
_NPIN = 15
_BS = 32
_AHEAD = 3
_RS = 64
_WS = 16
_NB = 3
_LEAD = 2


def _pin_positions(n, rows):
    pos = [round(i * (2 * rows - 16) / (n - 2) / 16) * 16 for i in range(n - 1)]
    return [(0, p) if p < rows else (2, p - rows) for p in pos]


@jax.jit
def pallas_standalone__depthwise_separable__vision_kernel(
    x: jax.Array,
    dw: jax.Array,
    pw: jax.Array,
):
    B, H, W, C = x.shape
    assert dw.shape == (1, 1, C) and pw.shape == (C, C) and C == 384
    k, L, ts, i0, fs, npin = _K, _L, _TS, _I0, _FS, _NPIN
    bs, ahead, rs, ws, NB, lead = _BS, _AHEAD, _RS, _WS, _NB, _LEAD
    G = B * H * W // (k * L)
    assert G * k * L == B * H * W
    Q = L // ts
    n = G * Q
    n2 = n - i0
    per_tile = 2 * ts // fs
    full, left = divmod(i0 * npin, per_tile)
    left = left // 2 * fs
    nb_a, nb = i0 // 2, n // 2
    ring = ahead + 1
    assert k % 2 == 0 and i0 % 2 == 0 and full + 1 < n2 and nb_a <= n2 - lead <= nb - NB
    assert all((NB + j + 1) * 2 <= i0 + lead + j for j in range(n2 - lead))
    pins = _pin_positions(npin, k * ts)

    def aligned(v):
        return v if isinstance(v, int) else pl.multiple_of(v, 16)

    def div(a, b):
        return a // b if isinstance(a, int) else lax.div(a, b)

    def rem(a, b):
        return a % b if isinstance(a, int) else lax.rem(a, b)

    def kernel(x_hbm, dw_hbm, pw_hbm, o_hbm, buf_a, buf_b, dw_ref, pw_ref, wsems):
        def hbm(ref, t, lo, size, s0=0, sn=k):
            rows = pl.ds(aligned(rem(t, Q) * ts + lo), size)
            return ref.at[div(t, Q), pl.ds(s0, sn), rows, :]

        def vmem(buf, slot, lo, size, s0=0, sn=k):
            return buf.at[pl.ds(slot * k + s0, sn), pl.ds(aligned(lo), size), :]

        def write(in_a, b, half, lo, size):
            t = 2 * b + half
            src = vmem(buf_a, t, lo, size) if in_a else vmem(buf_b, t - i0, lo, size)
            return pltpu.make_async_copy(
                src, hbm(o_hbm, t, lo, size), wsems.at[rem(b, NB)])

        def write_start(in_a, b):
            for half in range(2):
                for lo in range(0, ts, ws):
                    write(in_a, b, half, lo, ws).start()

        def write_wait(in_a, b):
            for half in range(2):
                write(in_a, b, half, 0, ts).wait()

        def compute(buf, slot):
            xt = buf[pl.ds(slot * k, k)].reshape(k * ts, C)
            y = jnp.dot(xt * dw_ref[0], pw_ref[...],
                        preferred_element_type=jnp.float32)
            buf[pl.ds(slot * k, k)] = y.astype(buf.dtype).reshape(k, ts, C)
            return y

        def read_phase(rsems):
            hi_sem, lo_sem, last_sem = (rsems.at[ring + i] for i in range(3))

            def read_a(t, lo, size):
                return pltpu.make_async_copy(
                    hbm(x_hbm, t, lo, size), vmem(buf_a, t, lo, size),
                    rsems.at[rem(t, ring)])

            def read_b(slot, lo, size, sem, *streams):
                return pltpu.make_async_copy(
                    hbm(x_hbm, i0 + slot, lo, size, *streams),
                    vmem(buf_b, slot, lo, size, *streams), sem)

            def start_tile_a(t):
                for lo in range(0, ts, bs):
                    read_a(t, lo, bs).start(priority=1)

            copy_dw = pltpu.make_async_copy(dw_hbm, dw_ref, lo_sem)
            copy_pw = pltpu.make_async_copy(pw_hbm, pw_ref, lo_sem)
            start_tile_a(0)
            copy_dw.start(priority=1)
            copy_pw.start(priority=1)
            for t in range(1, ahead):
                start_tile_a(t)
            copy_dw.wait()
            copy_pw.wait()

            rest = [read_b(full, left, ts - left, lo_sem)]
            rest += [read_b(slot, lo, rs, lo_sem)
                     for slot in range(full + 1, n2 - 1) for lo in range(0, ts, rs)]
            last = read_b(n2 - 1, 0, ts, last_sem)

            def step(t, carry):
                read_a(t, 0, ts).wait()

                @pl.when(t + ahead < i0)
                def _():
                    start_tile_a(t + ahead)

                @pl.when(t + ahead == i0)
                def _():
                    for c in rest + [last]:
                        c.start(priority=1)

                y = compute(buf_a, t)
                for i in range(npin):
                    if i > 0:
                        cb, r = pins[i - 1]
                        buf_b[n2 * k, pl.ds(0, 16), pl.ds(0, 128)] = (
                            y[r:r + 16, cb * 128:(cb + 1) * 128].astype(buf_b.dtype))
                    d = t * npin + i
                    read_b(div(d, per_tile), div(rem(d, per_tile), 2) * fs, fs, hi_sem,
                           rem(d, 2) * (k // 2), k // 2).start(priority=0)
                return carry

            lax.fori_loop(0, i0, step, 0)
            whole = buf_b.at[pl.ds(0, full * k)]
            pltpu.make_async_copy(whole, whole, hi_sem).wait()
            if left:
                read_b(full, 0, left, hi_sem).wait()
            for c in rest:
                c.wait()
            for b in range(NB):
                write_start(True, b)
            last.wait()

        pl.run_scoped(read_phase, pltpu.SemaphoreType.DMA((ring + 3,)))

        def step_a(j, carry):
            @pl.when(j >= 0)
            def _():
                write_wait(True, j)
                write_start(True, j + NB)

            compute(buf_b, j + lead)
            return carry

        def step_b(j, carry):
            @pl.when(j < nb_a)
            def _():
                write_wait(True, j)

            @pl.when(j >= nb_a)
            def _():
                write_wait(False, j)

            write_start(False, j + NB)
            compute(buf_b, j + lead)
            return carry

        def drain(j, carry):
            write_wait(False, j)
            write_start(False, j + NB)
            return carry

        lax.fori_loop(-lead, nb_a - NB, step_a, 0)
        lax.fori_loop(nb_a - NB, n2 - lead, step_b, 0)
        lax.fori_loop(n2 - lead, nb - NB, drain, 0)
        for b in range(nb - NB, nb):
            write_wait(False, b)

    out = pl.pallas_call(
        kernel,
        in_specs=[pl.BlockSpec(memory_space=pl.ANY)] * 3,
        out_specs=pl.BlockSpec(memory_space=pl.ANY),
        out_shape=jax.ShapeDtypeStruct((G, k, L, C), x.dtype),
        scratch_shapes=[
            pltpu.VMEM((i0 * k, ts, C), x.dtype),
            pltpu.VMEM((n2 * k + 1, ts, C), x.dtype),
            pltpu.VMEM(dw.shape, dw.dtype),
            pltpu.VMEM(pw.shape, pw.dtype),
            pltpu.SemaphoreType.DMA((NB,)),
        ],
        compiler_params=pltpu.CompilerParams(vmem_limit_bytes=120 * 1024 * 1024),
    )(x.reshape(G, k, L, C), dw, pw)
    return out.reshape(B, H, W, C)
```

```python
import jax
import jax.numpy as jnp
from jax import lax
import jax.experimental.pallas as pl
import jax.experimental.pallas.tpu as pltpu

_K = 6
_L = 2048
_TS = 128
_I0 = 98
_FS = 16
_NPIN = 15
_BS = 32
_AHEAD = 3
_RS = 64
_WS = 16
_NB = 3
_LEAD = 2


def _pin_positions(n, rows):
    pos = [round(i * (2 * rows - 16) / (n - 2) / 16) * 16 for i in range(n - 1)]
    return [(0, p) if p < rows else (2, p - rows) for p in pos]


@jax.jit
def pallas_standalone__depthwise_separable__vision_kernel(
    x: jax.Array,
    dw: jax.Array,
    pw: jax.Array,
):
    B, H, W, C = x.shape
    assert dw.shape == (1, 1, C) and pw.shape == (C, C) and C == 384
    k, L, ts, i0, fs, npin = _K, _L, _TS, _I0, _FS, _NPIN
    bs, ahead, rs, ws, NB, lead = _BS, _AHEAD, _RS, _WS, _NB, _LEAD
    G = B * H * W // (k * L)
    assert G * k * L == B * H * W
    Q = L // ts
    n = G * Q
    n2 = n - i0
    per_tile = 2 * ts // fs
    full, left = divmod(i0 * npin, per_tile)
    left = left // 2 * fs
    nb_a, nb = i0 // 2, n // 2
    ring = ahead + 1
    assert k % 2 == 0 and i0 % 2 == 0 and full + 1 < n2 and nb_a <= n2 - lead <= nb - NB
    assert all((NB + j + 1) * 2 <= i0 + lead + j for j in range(n2 - lead))
    pins = _pin_positions(npin, k * ts)

    def aligned(v):
        return v if isinstance(v, int) else pl.multiple_of(v, 16)

    def div(a, b):
        return a // b if isinstance(a, int) else lax.div(a, b)

    def rem(a, b):
        return a % b if isinstance(a, int) else lax.rem(a, b)

    def body(x_hbm, dw_hbm, pw_hbm, o_hbm, buf_a, buf_b, dw_ref, pw_ref, wsems):
        def hbm(ref, t, lo, size, s0=0, sn=k):
            rows = pl.ds(aligned(rem(t, Q) * ts + lo), size)
            return ref.at[div(t, Q), pl.ds(s0, sn), rows, :]

        def vmem(buf, slot, lo, size, s0=0, sn=k):
            return buf.at[pl.ds(slot * k + s0, sn), pl.ds(aligned(lo), size), :]

        def write(in_a, b, half, lo, size):
            t = 2 * b + half
            src = vmem(buf_a, t, lo, size) if in_a else vmem(buf_b, t - i0, lo, size)
            return pltpu.make_async_copy(
                src, hbm(o_hbm, t, lo, size), wsems.at[rem(b, NB)])

        def write_start(in_a, b):
            for half in range(2):
                for lo in range(0, ts, ws):
                    write(in_a, b, half, lo, ws).start()

        def write_wait(in_a, b):
            for half in range(2):
                write(in_a, b, half, 0, ts).wait()

        def compute(buf, slot):
            xt = buf[pl.ds(slot * k, k)].reshape(k * ts, C)
            y = jnp.dot(xt * dw_ref[0], pw_ref[...],
                        preferred_element_type=jnp.float32)
            buf[pl.ds(slot * k, k)] = y.astype(buf.dtype).reshape(k, ts, C)
            return y

        def read_phase(rsems):
            hi_sem, lo_sem, last_sem = (rsems.at[ring + i] for i in range(3))

            def read_a(t, lo, size):
                return pltpu.make_async_copy(
                    hbm(x_hbm, t, lo, size), vmem(buf_a, t, lo, size),
                    rsems.at[rem(t, ring)])

            def read_b(slot, lo, size, sem, *streams):
                return pltpu.make_async_copy(
                    hbm(x_hbm, i0 + slot, lo, size, *streams),
                    vmem(buf_b, slot, lo, size, *streams), sem)

            def start_tile_a(t):
                for lo in range(0, ts, bs):
                    read_a(t, lo, bs).start(priority=1)

            copy_dw = pltpu.make_async_copy(dw_hbm, dw_ref, lo_sem)
            copy_pw = pltpu.make_async_copy(pw_hbm, pw_ref, lo_sem)
            start_tile_a(0)
            copy_dw.start(priority=1)
            copy_pw.start(priority=1)
            for t in range(1, ahead):
                start_tile_a(t)
            copy_dw.wait()
            copy_pw.wait()

            rest = [read_b(full, left, ts - left, lo_sem)]
            rest += [read_b(slot, lo, rs, lo_sem)
                     for slot in range(full + 1, n2 - 1) for lo in range(0, ts, rs)]
            last = read_b(n2 - 1, 0, ts, last_sem)

            def step(t, carry):
                read_a(t, 0, ts).wait()

                @pl.when(t + ahead < i0)
                def _():
                    start_tile_a(t + ahead)

                @pl.when(t + ahead == i0)
                def _():
                    for c in rest + [last]:
                        c.start(priority=1)

                y = compute(buf_a, t)
                for i in range(npin):
                    if i > 0:
                        cb, r = pins[i - 1]
                        buf_b[n2 * k, pl.ds(0, 16), pl.ds(0, 128)] = (
                            y[r:r + 16, cb * 128:(cb + 1) * 128].astype(buf_b.dtype))
                    d = t * npin + i
                    read_b(div(d, per_tile), div(rem(d, per_tile), 2) * fs, fs, hi_sem,
                           rem(d, 2) * (k // 2), k // 2).start(priority=0)
                return carry

            lax.fori_loop(0, i0, step, 0)
            whole = buf_b.at[pl.ds(0, full * k)]
            pltpu.make_async_copy(whole, whole, hi_sem).wait()
            if left:
                read_b(full, 0, left, hi_sem).wait()
            for c in rest:
                c.wait()
            for b in range(NB):
                write_start(True, b)
            last.wait()

        pl.run_scoped(read_phase, pltpu.SemaphoreType.DMA((ring + 3,)))

        def step_a(j, carry):
            @pl.when(j >= 0)
            def _():
                write_wait(True, j)
                write_start(True, j + NB)

            compute(buf_b, j + lead)
            return carry

        def step_b(j, carry):
            @pl.when(j < nb_a)
            def _():
                write_wait(True, j)

            @pl.when(j >= nb_a)
            def _():
                write_wait(False, j)

            write_start(False, j + NB)
            compute(buf_b, j + lead)
            return carry

        def drain(j, carry):
            write_wait(False, j)
            write_start(False, j + NB)
            return carry

        lax.fori_loop(-lead, nb_a - NB, step_a, 0)
        lax.fori_loop(nb_a - NB, n2 - lead, step_b, 0)
        lax.fori_loop(n2 - lead, nb - NB, drain, 0)
        for b in range(nb - NB, nb):
            write_wait(False, b)

    def kernel(*refs):
        pl.run_scoped(lambda wsems: body(*refs, wsems),
                      pltpu.SemaphoreType.DMA((NB,)))

    out = pl.pallas_call(
        kernel,
        in_specs=[pl.BlockSpec(memory_space=pl.ANY)] * 3,
        out_specs=pl.BlockSpec(memory_space=pl.ANY),
        out_shape=jax.ShapeDtypeStruct((G, k, L, C), x.dtype),
        scratch_shapes=[
            pltpu.VMEM((i0 * k, ts, C), x.dtype),
            pltpu.VMEM((n2 * k + 1, ts, C), x.dtype),
            pltpu.VMEM(dw.shape, dw.dtype),
            pltpu.VMEM(pw.shape, pw.dtype),
        ],
        compiler_params=pltpu.CompilerParams(vmem_limit_bytes=120 * 1024 * 1024),
    )(x.reshape(G, k, L, C), dw, pw)
    return out.reshape(B, H, W, C)
```
